```python
import jax
import jax.numpy as jnp

def _softmax(x, axis=-1):
    return jax.nn.softmax(x, axis=axis)

def _gelu(x):
    return jax.nn.gelu(x, approximate=True)

def _silu(x):
    return jax.nn.silu(x)

def _sigmoid(x):
    return jax.nn.sigmoid(x)

def _layernorm(x, axis=-1, eps=1e-05):
    m = jnp.mean(x, axis=axis, keepdims=True)
    v = jnp.var(x, axis=axis, keepdims=True)
    return (x - m) / jnp.sqrt(v + eps)

def _scatter_add(tgt, idx, src, axis=0):
    return tgt.at[idx].add(src)

def _segment_sum(src, seg, n):
    return jax.ops.segment_sum(src, seg, n)

class _Rng:

    def __init__(self, key):
        self._k = key

    def _next(self):
        self._k, sub = jax.random.split(self._k)
        return sub

    def normal(self, shape):
        return jax.random.normal(self._next(), shape, dtype=jnp.bfloat16)

    def randint(self, lo, hi, shape):
        return jax.random.randint(self._next(), shape, lo, hi, dtype=jnp.int32)

    def uniform(self, shape, lo=0.0, hi=1.0):
        return jax.random.uniform(self._next(), shape, jnp.bfloat16, lo, hi)

    def permutation(self, n):
        return jax.random.permutation(self._next(), n)
kernel_name = 'sequential_preLN__ssm_conv_s4__mixer_gmlp__prompt'

def _fwd_setup_inputs():
    _rng = _Rng(jax.random.key(int.from_bytes(__import__("os").urandom(4), "little")))
    _w = lambda a: (lambda t: t.astype(jnp.bfloat16) if jnp.issubdtype(t.dtype, jnp.floating) else t)(jnp.asarray(a))

    def _A_setup():
        B, L, D, N = (1, 2048, 576, 128)
        A_re = -jnp.exp((lambda *s: _rng.normal(s) * 0.05)(D, N))
        A_im = jnp.pi * (lambda *s: _rng.normal(s) * 0.05)(D, N)
        B_re = (lambda *s: _rng.normal(s) * 0.05)(D, N)
        B_im = (lambda *s: _rng.normal(s) * 0.05)(D, N)
        C_re = (lambda *s: _rng.normal(s) * 0.05)(D, N)
        C_im = (lambda *s: _rng.normal(s) * 0.05)(D, N)
        log_dt = (lambda *s: _rng.normal(s) * 0.05)(D) * 0.5 - 4.0
        Dskip = (lambda *s: _rng.normal(s) * 0.05)(D)
        return {'u': _w((lambda *s: _rng.normal(s) * 0.05)(B, L, D)), 'A_re': _w(A_re), 'A_im': _w(A_im), 'B_re': _w(B_re), 'B_im': _w(B_im), 'C_re': _w(C_re), 'C_im': _w(C_im), 'log_dt': _w(log_dt), 'Dskip': _w(Dskip)}
    _A_in = _A_setup()

    def _B_setup():
        B, S, D, F = (1, 2048, 576, 4608)
        Fh = F // 2
        return {'x': _w((lambda *s: _rng.normal(s) * 0.05)(B, S, D)), 'w_in': _w((lambda *s: _rng.normal(s) * 0.05)(D, 2 * Fh)), 'w_sp': _w(0.01 * (lambda *s: _rng.normal(s) * 0.05)(S, S)), 'b_sp': _w(1.0 + 0.01 * (lambda *s: _rng.normal(s) * 0.05)(S)), 'w_out': _w((lambda *s: _rng.normal(s) * 0.05)(Fh, D))}
    _B_in = _B_setup()
    return {'A_u': _A_in['u'], 'A_A_re': _A_in['A_re'], 'A_A_im': _A_in['A_im'], 'A_B_re': _A_in['B_re'], 'A_B_im': _A_in['B_im'], 'A_C_re': _A_in['C_re'], 'A_C_im': _A_in['C_im'], 'A_log_dt': _A_in['log_dt'], 'A_Dskip': _A_in['Dskip'], 'B_x': _B_in['x'], 'B_w_in': _B_in['w_in'], 'B_w_sp': _B_in['w_sp'], 'B_b_sp': _B_in['b_sp'], 'B_w_out': _B_in['w_out']}

def _fwd_reference(A_u, A_A_re, A_A_im, A_B_re, A_B_im, A_C_re, A_C_im, A_log_dt, A_Dskip, B_x, B_w_in, B_w_sp, B_b_sp, B_w_out):

    def _A_ref(u, A_re, A_im, B_re, B_im, C_re, C_im, log_dt, Dskip):
        Bsz, L, D = u.shape
        dt = jnp.exp(log_dt)[:, None]
        A = A_re + 1j * A_im
        Bc = B_re + 1j * B_im
        Cc = C_re + 1j * C_im
        logdA = dt * A
        dB = dt * Bc
        l = (lambda x, dt: x.astype(dt))(jnp.arange(L), A_re.dtype)
        P = jnp.exp(logdA[:, :, None] * l[None, None, :])
        K = jnp.einsum('dn,dnl,dn->dl', Cc, P, dB).real
        L2 = 2 * L
        Kp = jnp.pad(K, ((0, 0), (0, L)))
        up = (lambda x, *d: x.transpose(*d))(u, 0, 2, 1)
        up = jnp.pad(up, ((0, 0), (0, 0), (0, L)))
        Kf = (lambda x, axes=(-2, -1): jnp.fft.rfft2(x.astype(jnp.float32), axes=axes))(Kp[:, None, :], axes=(-2, -1))
        Uf = (lambda x, axes=(-2, -1): jnp.fft.rfft2(x.astype(jnp.float32), axes=axes))(up[:, :, None, :], axes=(-2, -1))
        Yf = Uf * Kf[None, :, :, :]
        y = (lambda x, s, axes=(-2, -1): jnp.fft.irfft2(x, s=s, axes=axes).astype(jnp.bfloat16))(Yf, (1, L2), axes=(-2, -1))[:, :, 0, :L]
        y = (lambda x, *d: x.transpose(*d))(y, 0, 2, 1) + u * Dskip[None, None, :]
        return y

    def _B_ref(x, w_in, w_sp, b_sp, w_out):
        B, S, D = x.shape
        F = w_in.shape[-1]
        Fh = F // 2
        z = _gelu(jnp.einsum('bsd,df->bsf', x, w_in))
        z1 = z[..., :Fh].copy()
        z2 = _layernorm(z[..., Fh:], axis=-1)
        g = jnp.einsum('ts,bsf->btf', w_sp, z2) + b_sp[None, :, None]
        return jnp.einsum('bsf,fd->bsd', z1 * g, w_out)
    x = A_u
    h = x + _A_ref(_layernorm(x, axis=-1), A_A_re, A_A_im, A_B_re, A_B_im, A_C_re, A_C_im, A_log_dt, A_Dskip)
    h2 = h + _B_ref(_layernorm(h, axis=-1), B_w_in, B_w_sp, B_b_sp, B_w_out)
    return h2

def setup_inputs():
    _inp = _fwd_setup_inputs()
    _gk = jax.random.fold_in(jax.random.key(int.from_bytes(__import__("os").urandom(4), "little")), 2 ** 31 - 1)
    _shapes = [[1, 2048, 576]]
    _dtypes = ['bfloat16']
    _gks = jax.random.split(_gk, len(_shapes))
    _gs = [jax.random.normal(k, s, dtype=jnp.dtype(d)) * 0.05 for k, s, d in zip(_gks, _shapes, _dtypes)]
    _inp['grad_out'] = _gs[0]
    return _inp

def reference(A_u, A_A_re, A_A_im, A_B_re, A_B_im, A_C_re, A_C_im, A_log_dt, A_Dskip, B_w_in, B_w_sp, B_b_sp, B_w_out, B_x, grad_out):
    _const = dict(B_x=B_x)

    def _f(*_d):
        return _fwd_reference(**{'A_u': _d[0], 'A_A_re': _d[1], 'A_A_im': _d[2], 'A_B_re': _d[3], 'A_B_im': _d[4], 'A_C_re': _d[5], 'A_C_im': _d[6], 'A_log_dt': _d[7], 'A_Dskip': _d[8], 'B_w_in': _d[9], 'B_w_sp': _d[10], 'B_b_sp': _d[11], 'B_w_out': _d[12], **_const})
    _out, _vjp = jax.vjp(_f, A_u, A_A_re, A_A_im, A_B_re, A_B_im, A_C_re, A_C_im, A_log_dt, A_Dskip, B_w_in, B_w_sp, B_b_sp, B_w_out)
    _grads = _vjp(grad_out)
    _out0 = jnp.asarray(_out)
    return (_out0, *[jnp.asarray(_g) for _g in _grads])
```

```python
import numpy as np
import jax
import jax.numpy as jnp
from jax import lax
import jax.experimental.pallas as pl
import jax.experimental.pallas.tpu as pltpu

L = 2048
D = 576
DP = 640
N = 128
FH = 2304
FF = 4608
NF = 4096
TM = 256
TF = 512
NBLK = 41
J = NBLK * 16
EPS = 1e-5
_BLOCKS = [(0, hi) for hi in range(16)] + [(s, hi) for s in (1, 2, 3) for hi in range(8, 16)] + [(4, 8)]
F32 = jnp.float32
BF16 = jnp.bfloat16


def _consts():
    k = np.arange(L, dtype=np.int64)
    kn = (k[:, None] * k[None, :]) % NF
    ang = 2.0 * np.pi * kn.astype(np.float64) / NF
    C = np.cos(ang)
    S = np.sin(ang)
    S[0, :] = np.where(k % 2 == 0, 1.0, -1.0)
    Fm = np.concatenate([C, S], axis=0)
    q = np.arange(L, dtype=np.float32).astype(BF16).astype(np.int64)
    pos = {}
    for b, (s, hi) in enumerate(_BLOCKS):
        for lo in range(16):
            pos.setdefault((16 * hi + lo) << s, b * 16 + lo)
    E = np.zeros((L, J), np.float64)
    E[np.arange(L), [pos[int(v)] for v in q]] = 1.0
    FE = Fm @ E
    return (jnp.asarray(Fm.astype(np.float32)).astype(BF16),
            jnp.asarray(FE.astype(np.float32)).astype(BF16),
            jnp.asarray(np.ascontiguousarray(FE.T).astype(np.float32)).astype(BF16))


def _dot(a, b):
    return jnp.dot(a, b, preferred_element_type=F32)


def _dot_nt(a, b):
    return lax.dot_general(a, b, (((1,), (1,)), ((), ())), preferred_element_type=F32)


def _dot_tn(a, b):
    return lax.dot_general(a, b, (((0,), (0,)), ((), ())), preferred_element_type=F32)


def _ln(x):
    m = jnp.mean(x, axis=-1, keepdims=True)
    xc = x - m
    v = jnp.mean(xc * xc, axis=-1, keepdims=True)
    r = lax.rsqrt(v + EPS)
    return xc * r, r


def _ln_bwd(dy, yhat, r):
    return r * (dy - jnp.mean(dy, axis=-1, keepdims=True)
                - yhat * jnp.mean(dy * yhat, axis=-1, keepdims=True))


_GC = 0.7978845608028654


def _gelu_and_grad(x):
    x2 = x * x
    t = jnp.tanh(_GC * x * (1.0 + 0.044715 * x2))
    g = 0.5 * x * (1.0 + t)
    dg = 0.5 * (1.0 + t) + 0.5 * x * (1.0 - t * t) * _GC * (1.0 + 3 * 0.044715 * x2)
    return g, dg


def _cmul(ar, ai, br, bi):
    return ar * br - ai * bi, ar * bi + ai * br


def _tables(ar, ai):
    er = jnp.exp(ar)
    p = [(er * jnp.cos(ai), er * jnp.sin(ai))]
    for _ in range(11):
        p.append(_cmul(*p[-1], *p[-1]))
    one = (jnp.ones_like(ar), jnp.zeros_like(ar))
    Y, X = {}, {}
    for s in range(5):
        ys = [one]
        for _ in range(15 if s < 4 else 0):
            ys.append(_cmul(*ys[-1], *p[s]))
        Y[s] = ys
        if s == 0:
            xs = {0: one}
            for hi in range(1, 16):
                xs[hi] = _cmul(*xs[hi - 1], *p[4])
        else:
            xs = {8: p[s + 7]}
            for hi in range(9, 16 if s < 4 else 9):
                xs[hi] = _cmul(*xs[hi - 1], *p[s + 4])
        X[s] = xs
    return Y, X


def _kernel(x_ref, go_ref, are_ref, aim_ref, bre_ref, bim_ref, cre_ref, cim_ref, ldt_ref, dsk_ref,
            win_ref, wsp_ref, bsp_ref, wout_ref, f_hbm, fe_ref, fet_ref,
            h2_ref, dx_ref, dare_ref, daim_ref, dbre_ref, dbim_ref, dcre_ref, dcim_ref, dldt_ref,
            ddsk_ref, dwin_ref, dwsp_ref, dbsp_ref, dwout_ref,
            u_s, h_s, b_s, dh_s, uf_s, kf_s, yw_s, acc_s, fbuf, sems):

    def params(nt, dt):
        sl = (pl.ds(pl.multiple_of(nt * 8, 8), 8), pl.ds(pl.multiple_of(dt * 128, 128), 128))
        dtv = jnp.exp(ldt_ref[:, sl[1]].astype(F32)).astype(BF16).astype(F32)
        ar = dtv * are_ref[sl].astype(F32)
        ai = dtv * aim_ref[sl].astype(F32)
        cbr, cbi = _cmul(cre_ref[sl].astype(F32), cim_ref[sl].astype(F32),
                         dtv * bre_ref[sl].astype(F32), dtv * bim_ref[sl].astype(F32))
        return sl, ar, ai, cbr, cbi

    def stream_f(body):
        def cp(i, slot):
            return pltpu.make_async_copy(f_hbm.at[pl.ds(i * TF, TF)], fbuf.at[slot], sems.at[slot])
        cp(0, 0).start()

        def step(i, c):
            slot = i % 2

            @pl.when(i + 1 < NF // TF)
            def _():
                cp(i + 1, 1 - slot).start()
            cp(i, slot).wait()
            body(i, fbuf[slot])
            return c
        lax.fori_loop(0, NF // TF, step, 0)

    def fwd_dft(src_ref, dst_ref):
        def body(i, f):
            dst_ref[pl.ds(pl.multiple_of(i * TF, TF), TF), :] = _dot(f, src_ref[...]).astype(BF16)
        stream_f(body)

    def inv_dft():
        nh = L // TF

        def body(i, f):
            @pl.when(i < nh)
            def _():
                acc_s[pl.ds(pl.multiple_of(i * TF, TF), TF), :] = _dot(f, yw_s[0:L, :])

            @pl.when(i >= nh)
            def _():
                r0 = pl.multiple_of((i - nh) * TF, TF)
                sp = _dot(f, yw_s[L:NF, :])
                n = r0 + lax.broadcasted_iota(jnp.int32, (TF, 1), 0)
                nyq = yw_s[L:L + 16, :].astype(F32)[0:1, :]
                sgn = (1 - 2 * (n % 2)).astype(F32)
                sp = jnp.where(n == 0, 0.0, sp) + sgn * nyq
                acc_s[pl.ds(r0, TF), :] += sp
        stream_f(body)

    def spec_prod(a_ref, b_ref, conj):
        for c in range(L // TF):
            r = slice(c * TF, (c + 1) * TF)
            s = slice(L + c * TF, L + (c + 1) * TF)
            ar_, as_ = a_ref[r, :].astype(F32), a_ref[s, :].astype(F32)
            br_, bs_ = b_ref[r, :].astype(F32), b_ref[s, :].astype(F32)
            ss = as_ * bs_
            row0 = (lax.broadcasted_iota(jnp.int32, (TF, 1), 0) + c * TF) == 0
            ssz = jnp.where(row0, 0.0, ss)
            if conj:
                yr = ar_ * br_ + ssz
                ys = jnp.where(row0, ss, as_ * br_ - ar_ * bs_)
            else:
                yr = ar_ * br_ - ssz
                ys = jnp.where(row0, ss, ar_ * bs_ + as_ * br_)
            w = jnp.where(row0, 1.0 / NF, 2.0 / NF)
            yw_s[r, :] = (yr * w).astype(BF16)
            yw_s[s, :] = (ys * w).astype(BF16)

    u0, _ = _ln(x_ref[...].astype(F32))
    u_s[...] = u0.astype(BF16)

    def kgen(kpart, fe_v):
        cpe = pltpu.make_async_copy(fe_ref, fe_v, sems.at[2])
        cpe.start()
        def tile(it, c):
            dt, nt = it // 16, it % 16
            sl, ar, ai, cbr, cbi = params(nt, dt)
            Y, X = _tables(ar, ai)
            for b, (s, hi) in enumerate(_BLOCKS):
                xr, xi = _cmul(cbr, cbi, *X[s][hi])
                for lo in range(16):
                    j = b * 16 + lo
                    if lo < len(Y[s]):
                        v = xr * Y[s][lo][0] - xi * Y[s][lo][1]
                    else:
                        v = jnp.zeros_like(xr)
                    kpart[j, :, sl[1]] = jnp.where(nt == 0, 0.0, kpart[j, :, sl[1]]) + v
            return c
        lax.fori_loop(0, 5 * 16, tile, 0)
        kq = jnp.sum(kpart[...], axis=1)[:, :D].astype(BF16)
        cpe.wait()
        for c in range(NF // TF):
            kf_s[c * TF:(c + 1) * TF, :] = _dot(fe_v[c * TF:(c + 1) * TF, :], kq).astype(BF16)
    pl.run_scoped(kgen, pltpu.VMEM((J, 8, DP), F32), pltpu.VMEM((NF, J), BF16))

    fwd_dft(u_s, uf_s)
    spec_prod(uf_s, kf_s, False)
    inv_dft()
    dsk = dsk_ref[...].astype(F32)
    yb = acc_s[...].astype(BF16).astype(F32) + (u_s[...].astype(F32) * dsk).astype(BF16).astype(F32)
    hh = (x_ref[...].astype(F32) + yb.astype(BF16).astype(F32)).astype(BF16)
    h_s[...] = hh
    b_s[...] = _ln(hh.astype(F32))[0].astype(BF16)

    def mlp(pre_s, z2_s, r2_s, dg_s, dwo_s, ob1, ob2):
        def rows(i):
            return pl.ds(pl.multiple_of(i * TM, TM), TM)

        def pa(i, c):
            r = rows(i)
            pre = _dot(b_s[r, :], win_ref[...]).astype(BF16)
            pre_s[r, :] = pre
            z2 = _gelu_and_grad(pre[:, FH:].astype(F32))[0].astype(BF16).astype(F32)
            z2n, r2 = _ln(z2)
            z2_s[r, :] = z2n.astype(BF16)
            r2_s[r, :] = r2
            return c
        lax.fori_loop(0, L // TM, pa, 0)

        def pb(i, c):
            r = rows(i)
            g = (_dot(wsp_ref[r, :], z2_s[...]).astype(BF16).astype(F32)
                 + bsp_ref[r, :].astype(F32)).astype(BF16).astype(F32)
            z1, gp1 = _gelu_and_grad(pre_s[r, 0:FH].astype(F32))
            z1 = z1.astype(BF16).astype(F32)
            zg = (z1 * g).astype(BF16)
            go = go_ref[r, :]
            h2_ref[r, :] = (h_s[r, :].astype(F32)
                            + _dot(zg, wout_ref[...]).astype(BF16).astype(F32)).astype(BF16)
            dzg = _dot_nt(go, wout_ref[...]).astype(BF16).astype(F32)
            dwo_s[...] = jnp.where(i == 0, 0.0, dwo_s[...]) + _dot_tn(zg, go)
            dg = dzg * z1
            dbsp_ref[r, :] = jnp.sum(dg, axis=-1, keepdims=True).astype(BF16)
            dgb = dg.astype(BF16)
            dg_s[r, :] = dgb
            dwsp = _dot_nt(dgb, z2_s[...]).astype(BF16)

            @pl.when(i > 0)
            def _():
                pltpu.make_async_copy(ob1, dwsp_ref.at[r], sems.at[2]).wait()
            ob1[...] = dwsp
            pltpu.make_async_copy(ob1, dwsp_ref.at[r], sems.at[2]).start()
            pre_s[r, 0:FH] = (dzg * g * gp1).astype(BF16)
            return c
        lax.fori_loop(0, L // TM, pb, 0)
        pltpu.make_async_copy(ob1, dwsp_ref.at[pl.ds(0, TM)], sems.at[2]).wait()
        dwout_ref[...] = dwo_s[...].astype(BF16)

        def pc(i, c):
            r = rows(i)
            dz2 = _dot_tn(wsp_ref[:, r], dg_s[...])
            dzz = _ln_bwd(dz2, z2_s[r, :].astype(F32), r2_s[r, :])
            gp2 = _gelu_and_grad(pre_s[r, FH:FF].astype(F32))[1]
            pre_s[r, FH:FF] = (dzz * gp2).astype(BF16)
            db = _dot_nt(pre_s[r, :], win_ref[...])
            bh, rh = _ln(h_s[r, :].astype(F32))
            dh_s[r, :] = (go_ref[r, :].astype(F32) + _ln_bwd(db, bh, rh)).astype(BF16)
            return c
        lax.fori_loop(0, L // TM, pc, 0)

        def pd(i, c):
            cs = pl.ds(pl.multiple_of(i * 512, 512), 512)
            dwin = _dot_tn(b_s[...], pre_s[:, cs]).astype(BF16)

            @pl.when(i > 0)
            def _():
                pltpu.make_async_copy(ob2, dwin_ref.at[:, cs], sems.at[2]).wait()
            ob2[...] = dwin
            pltpu.make_async_copy(ob2, dwin_ref.at[:, cs], sems.at[2]).start()
            return c
        lax.fori_loop(0, FF // 512, pd, 0)
        pltpu.make_async_copy(ob2, dwin_ref.at[:, pl.ds(0, 512)], sems.at[2]).wait()

    pl.run_scoped(mlp, pltpu.VMEM((L, FF), BF16), pltpu.VMEM((L, FH), BF16), pltpu.VMEM((L, 1), F32),
                  pltpu.VMEM((L, FH), BF16), pltpu.VMEM((FH, D), F32), pltpu.VMEM((TM, L), BF16), pltpu.VMEM((D, 512), BF16))

    def ssm_bwd(dyf_s, dkq_s, g_s, fet_v):
        cpe = pltpu.make_async_copy(fet_ref, fet_v, sems.at[2])
        cpe.start()
        fwd_dft(dh_s, dyf_s)
        spec_prod(dyf_s, uf_s, True)
        dkq_s[...] = jnp.zeros((J, DP), F32)
        cpe.wait()
        dkq_s[:, 0:D] = _dot(fet_v[...], yw_s[...])
        spec_prod(dyf_s, kf_s, True)
        inv_dft()
        dh = dh_s[...].astype(F32)
        uu = u_s[...].astype(F32)
        ddsk_ref[...] = jnp.sum(dh * uu, axis=0, keepdims=True).astype(BF16)
        du = acc_s[...] + dh * dsk
        _, rx = _ln(x_ref[...].astype(F32))
        dx_ref[...] = (dh + _ln_bwd(du, uu, rx)).astype(BF16)

        def tile(it, c):
            dt, nt = it // 16, it % 16
            sl, ar, ai, cbr, cbi = params(nt, dt)
            Y, X = _tables(ar, ai)
            z = jnp.zeros_like(ar)
            g0r, g0i, g1r, g1i = z, z, z, z
            for b, (s, hi) in enumerate(_BLOCKS):
                tr, ti, tpr, tpi = z, z, z, z
                for lo in range(len(Y[s])):
                    dk = dkq_s[pl.ds(b * 16 + lo, 1), sl[1]]
                    yr, yi = Y[s][lo]
                    tr, ti = tr + dk * yr, ti + dk * yi
                    if lo:
                        dl = dk * float(lo << s)
                        tpr, tpi = tpr + dl * yr, tpi + dl * yi
                qh = float((16 * hi) << s)
                xr, xi = X[s][hi]
                pr, pi_ = _cmul(xr, xi, tr, ti)
                g0r, g0i = g0r + pr, g0i + pi_
                pr, pi_ = _cmul(xr, xi, qh * tr + tpr, qh * ti + tpi)
                g1r, g1i = g1r + pr, g1i + pi_
            g_s[0, sl[0], sl[1]] = g0r
            g_s[1, sl[0], sl[1]] = g0i
            g_s[2, sl[0], sl[1]] = g1r
            g_s[3, sl[0], sl[1]] = g1i
            return c
        lax.fori_loop(0, 5 * 16, tile, 0)

        dtv = jnp.exp(ldt_ref[...].astype(F32)).astype(BF16).astype(F32)
        are, aim = are_ref[...].astype(F32), aim_ref[...].astype(F32)
        bre, bim = bre_ref[...].astype(F32), bim_ref[...].astype(F32)
        cre, cim = cre_ref[...].astype(F32), cim_ref[...].astype(F32)
        dbr, dbi = dtv * bre, dtv * bim
        cbr, cbi = _cmul(cre, cim, dbr, dbi)
        dcbr, dcbi = g_s[0], -g_s[1]
        t_r, t_i = _cmul(cbr, cbi, g_s[2], g_s[3])
        dar, dai = t_r, -t_i
        dcr, dci = _cmul(dbr, -dbi, dcbr, dcbi)
        ddbr, ddbi = _cmul(cre, -cim, dcbr, dcbi)
        dare_ref[...] = (dtv * dar).astype(BF16)
        daim_ref[...] = (dtv * dai).astype(BF16)
        dbre_ref[...] = (dtv * ddbr).astype(BF16)
        dbim_ref[...] = (dtv * ddbi).astype(BF16)
        dcre_ref[...] = dcr.astype(BF16)
        dcim_ref[...] = dci.astype(BF16)
        ddt = jnp.sum(bre * ddbr + bim * ddbi + are * dar + aim * dai, axis=0, keepdims=True)
        dldt_ref[...] = (ddt * dtv).astype(BF16)

    pl.run_scoped(ssm_bwd, pltpu.VMEM((NF, D), BF16), pltpu.VMEM((J, DP), F32),
                  pltpu.VMEM((4, N, DP), F32), pltpu.VMEM((J, NF), BF16))


@jax.jit
def pallas_sequential_preLN__ssm_conv_s4__mixer_gmlp__prompt_kernel(
    A_u, A_A_re, A_A_im, A_B_re, A_B_im, A_C_re, A_C_im, A_log_dt, A_Dskip,
    B_x, B_w_in, B_w_sp, B_b_sp, B_w_out, grad_out,
):
    fm, fe, fet = _consts()
    tp = lambda a: jnp.pad(a.T, ((0, 0), (0, DP - D)))
    ins = (A_u.reshape(L, D), grad_out.reshape(L, D), tp(A_A_re), tp(A_A_im), tp(A_B_re), tp(A_B_im),
           tp(A_C_re), tp(A_C_im), jnp.pad(A_log_dt.reshape(1, D), ((0, 0), (0, DP - D))),
           A_Dskip.reshape(1, D), B_w_in, B_w_sp, B_b_sp.reshape(L, 1), B_w_out, fm, fe, fet)
    vm = pl.BlockSpec(memory_space=pltpu.VMEM)
    an = pl.BlockSpec(memory_space=pl.ANY)
    in_specs = [vm] * 14 + [an] * 3
    out_specs = tuple([vm] * 10 + [an, an, vm, vm])
    sd = jax.ShapeDtypeStruct
    out_shape = (sd((L, D), BF16), sd((L, D), BF16)) + (sd((N, DP), BF16),) * 6 + (
        sd((1, DP), BF16), sd((1, D), BF16), sd((D, FF), BF16), sd((L, L), BF16), sd((L, 1), BF16),
        sd((FH, D), BF16))
    outs = pl.pallas_call(
        _kernel,
        out_shape=out_shape,
        in_specs=in_specs,
        out_specs=out_specs,
        scratch_shapes=[
            pltpu.VMEM((L, D), BF16), pltpu.VMEM((L, D), BF16), pltpu.VMEM((L, D), BF16),
            pltpu.VMEM((L, D), BF16), pltpu.VMEM((NF, D), BF16), pltpu.VMEM((NF, D), BF16),
            pltpu.VMEM((NF, D), BF16), pltpu.VMEM((L, D), F32), pltpu.VMEM((2, TF, L), BF16),
            pltpu.SemaphoreType.DMA((3,)),
        ],
        compiler_params=pltpu.CompilerParams(vmem_limit_bytes=127 * 1024 * 1024),
    )(*ins)
    h2, dx, dare, daim, dbre, dbim, dcre, dcim, dldt, ddsk, dwin, dwsp, dbsp, dwout = outs
    ut = lambda a: a[:, :D].T
    return (h2.reshape(1, L, D), dx.reshape(1, L, D), ut(dare), ut(daim), ut(dbre), ut(dbim), ut(dcre),
            ut(dcim), dldt[0, :D], ddsk.reshape(D), dwin, dwsp, dbsp.reshape(L), dwout)
```

```python
import numpy as np
import jax
import jax.numpy as jnp
from jax import lax
import jax.experimental.pallas as pl
import jax.experimental.pallas.tpu as pltpu

L = 2048
D = 576
DP = 640
N = 128
FH = 2304
FF = 4608
NF = 4096
TM = 256
TF = 512
NBLK = 41
J = NBLK * 16
EPS = 1e-5
_BLOCKS = [(0, hi) for hi in range(16)] + [(s, hi) for s in (1, 2, 3) for hi in range(8, 16)] + [(4, 8)]
F32 = jnp.float32
BF16 = jnp.bfloat16


H = L // 2


def _consts():
    k = np.arange(H, dtype=np.int64)
    ang = 2.0 * np.pi * ((k[:, None] * k[None, :]) % L).astype(np.float64) / L
    S = np.sin(ang)
    S[0, :] = np.where(k % 2 == 0, 1.0, -1.0)
    F2 = np.concatenate([np.cos(ang), S], axis=0)
    n = np.arange(L, dtype=np.int64)
    kp = k.copy()
    kq = L - k
    kps = k.copy()
    kps[0] = H
    kqs = L - k
    kqs[0] = H
    an = lambda kk: 2.0 * np.pi * ((kk[:, None] * n[None, :]) % NF).astype(np.float64) / NF
    Gps = np.sin(an(kps))
    Gps[0] = np.cos(an(kps))[0]
    G = np.concatenate([np.cos(an(kp)), Gps, np.cos(an(kq)), np.sin(an(kqs))], axis=0)
    q = np.arange(L, dtype=np.float32).astype(BF16).astype(np.int64)
    pos = {}
    for b, (s, hi) in enumerate(_BLOCKS):
        for lo in range(16):
            pos.setdefault((16 * hi + lo) << s, b * 16 + lo)
    E = np.zeros((L, J), np.float64)
    E[np.arange(L), [pos[int(v)] for v in q]] = 1.0
    FE = G @ E
    w = np.full((NF, 1), 2.0 / NF)
    w[0] = w[L] = 1.0 / NF
    bf = lambda a: jnp.asarray(np.ascontiguousarray(a).astype(np.float32)).astype(BF16)
    return bf(F2), bf(FE), bf((FE * w).T)


def _dot(a, b):
    return jnp.dot(a, b, preferred_element_type=F32)


def _dot_nt(a, b):
    return lax.dot_general(a, b, (((1,), (1,)), ((), ())), preferred_element_type=F32)


def _dot_tn(a, b):
    return lax.dot_general(a, b, (((0,), (0,)), ((), ())), preferred_element_type=F32)


def _ln(x):
    m = jnp.mean(x, axis=-1, keepdims=True)
    xc = x - m
    v = jnp.mean(xc * xc, axis=-1, keepdims=True)
    r = lax.rsqrt(v + EPS)
    return xc * r, r


def _ln_bwd(dy, yhat, r):
    return r * (dy - jnp.mean(dy, axis=-1, keepdims=True)
                - yhat * jnp.mean(dy * yhat, axis=-1, keepdims=True))


_GC = 0.7978845608028654


def _gelu_and_grad(x):
    x2 = x * x
    t = jnp.tanh(_GC * x * (1.0 + 0.044715 * x2))
    g = 0.5 * x * (1.0 + t)
    dg = 0.5 * (1.0 + t) + 0.5 * x * (1.0 - t * t) * _GC * (1.0 + 3 * 0.044715 * x2)
    return g, dg


def _cmul(ar, ai, br, bi):
    return ar * br - ai * bi, ar * bi + ai * br


def _blocks(ar, ai, xr0, xi0):
    er = jnp.exp(ar)
    p = [(er * jnp.cos(ai), er * jnp.sin(ai))]
    for _ in range(11):
        p.append(_cmul(*p[-1], *p[-1]))
    b = 0
    for s in range(5):
        ys = [None]
        for lo in range(1, 16 if s < 4 else 1):
            ys.append(p[s] if lo == 1 else _cmul(*ys[-1], *p[s]))
        x = (xr0, xi0) if s == 0 else (_cmul(xr0, xi0, *p[s + 7]) if xr0 is not None else p[s + 7])
        his = range(16) if s == 0 else (range(8, 16) if s < 4 else range(8, 9))
        for hi in his:
            if hi != his[0]:
                x = _cmul(*x, *p[s + 4])
            yield b, s, hi, ys, x
            b += 1


def _kernel(x_ref, go_ref, are_ref, aim_ref, bre_ref, bim_ref, cre_ref, cim_ref, ldt_ref, dsk_ref,
            win_h, wsp_h, bsp_ref, wout_h, got_h, f_ref, fe_ref, fet_ref,
            h2_ref, dx_ref, dare_ref, daim_ref, dbre_ref, dbim_ref, dcre_ref, dcim_ref, dldt_ref,
            ddsk_ref, dwin_ref, dwsp_ref, dbsp_ref, dwout_ref,
            u_s, h_s, b_s, dh_s, uf_s, kf_s, yw_s, acc_s, sems, win_ref, wsp_ref, wout_ref, got_ref):
    wcp = [pltpu.make_async_copy(a, b, sems.at[3 + i]) for i, (a, b) in enumerate(
        ((win_h, win_ref), (wsp_h, wsp_ref), (wout_h, wout_ref), (got_h, got_ref)))]
    for c_ in wcp:
        c_.start()

    def params(nt, dt):
        sl = (pl.ds(pl.multiple_of(nt * 8, 8), 8), pl.ds(pl.multiple_of(dt * 128, 128), 128))
        dtv = jnp.exp(ldt_ref[:, sl[1]].astype(F32)).astype(BF16).astype(F32)
        ar = dtv * are_ref[sl].astype(F32)
        ai = dtv * aim_ref[sl].astype(F32)
        cbr, cbi = _cmul(cre_ref[sl].astype(F32), cim_ref[sl].astype(F32),
                         dtv * bre_ref[sl].astype(F32), dtv * bim_ref[sl].astype(F32))
        return sl, ar, ai, cbr, cbi

    def acc_st(rs, v):
        for c in range(4):
            acc_s[c, rs, :] = v[:, c * 128:(c + 1) * 128]
        acc_s[4, rs, 0:64] = v[:, 512:D]

    def acc_ld(rs):
        return jnp.concatenate([acc_s[c, rs, :] for c in range(4)] + [acc_s[4, rs, 0:64]], axis=1)

    allr = pl.ds(0, L)
    CH = 256

    def chunk(i):
        r0 = pl.multiple_of(i * CH, CH)
        k = lax.broadcasted_iota(jnp.int32, (CH, 1), 0) + r0
        th = k.astype(F32) * (2.0 * np.pi / NF)
        return (lambda o: pl.ds(o + r0, CH)), k, k == 0, jnp.cos(th), jnp.sin(th)

    def fwd_dft(dst_ref):
        xe = acc_ld(pl.ds(0, H, stride=2)).astype(BF16)
        xo = acc_ld(pl.ds(1, H, stride=2)).astype(BF16)

        def body(i, c):
            rs, _, row0, tc, ts = chunk(i)
            fc, fs = f_ref[rs(0), :], f_ref[rs(H), :]
            er, es, or_, os_ = _dot(fc, xe), _dot(fs, xe), _dot(fc, xo), _dot(fs, xo)
            tr = tc * or_ - ts * os_
            tq = tc * os_ + ts * or_
            dst_ref[rs(0), :] = (er + tr).astype(BF16)
            dst_ref[rs(H), :] = jnp.where(row0, es, es + tq).astype(BF16)
            dst_ref[rs(L), :] = (er - tr).astype(BF16)
            dst_ref[rs(L + H), :] = jnp.where(row0, os_, tq - es).astype(BF16)
            return c
        lax.fori_loop(0, H // CH, body, 0)

    def inv_dft():
        def body(i, c):
            rs, k, row0, _, _ = chunk(i)
            sgn = (1 - 2 * (k % 2)).astype(F32)
            for par in range(2):
                o = par * L
                cp_ = _dot(f_ref[rs(0), :], yw_s[o:o + H, :])
                sp = _dot(f_ref[rs(H), :], yw_s[o + H:o + L, :])
                nyq = yw_s[o + H:o + H + 16, :].astype(F32)[0:1, :]
                acc_st(pl.ds(2 * CH * i + par, CH, stride=2), cp_ + jnp.where(row0, 0.0, sp) + sgn * nyq)
            return c
        lax.fori_loop(0, H // CH, body, 0)

    def spec_prod(a_ref, b_ref, conj, for_inv):
        sg = 1.0 if conj else -1.0

        def cx(ar_, as_, br_, bs_):
            return ar_ * br_ + sg * (as_ * bs_), as_ * br_ - sg * (ar_ * bs_)

        def body(i, c):
            rs, _, row0, tc, ts = chunk(i)
            apr, aps, aqr, aqs = [a_ref[rs(j * H), :].astype(F32) for j in range(4)]
            bpr, bps, bqr, bqs = [b_ref[rs(j * H), :].astype(F32) for j in range(4)]
            pr, ps = cx(apr, aps, bpr, bps)
            qr, qs = cx(aqr, aqs, bqr, bqs)
            nr, ns = cx(aps, aqs, bps, bqs)
            pr = jnp.where(row0, apr * bpr, pr)
            qr = jnp.where(row0, aqr * bqr, qr)
            ps = jnp.where(row0, nr, ps)
            qs = jnp.where(row0, ns, qs)
            if for_inv:
                w = jnp.where(row0, 1.0 / NF, 2.0 / NF)
                dr, ds_ = pr - qr, ps + qs
                outs = ((pr + qr) * w, jnp.where(row0, ps, ps - qs) * (2.0 / NF),
                        (dr * tc + jnp.where(row0, 0.0, ds_ * ts)) * w,
                        jnp.where(row0, qs, ds_ * tc - dr * ts) * (2.0 / NF))
            else:
                outs = (pr, ps, qr, qs)
            for j in range(4):
                yw_s[rs(j * H), :] = outs[j].astype(BF16)
            return c
        lax.fori_loop(0, H // CH, body, 0)

    u0, _ = _ln(x_ref[...].astype(F32))
    u_s[...] = u0.astype(BF16)
    acc_st(allr, u0.astype(BF16).astype(F32))

    def kgen(kpart, fe_v):
        cpe = pltpu.make_async_copy(fe_ref, fe_v, sems.at[2])
        cpe.start()
        def tile(it, c):
            dt, nt = it // 16, it % 16
            sl, ar, ai, cbr, cbi = params(nt, dt)
            for b, s, hi, ys, (xr, xi) in _blocks(ar, ai, cbr, cbi):
                for lo in range(len(ys)):
                    v = xr if lo == 0 else xr * ys[lo][0] - xi * ys[lo][1]
                    kpart[b * 16 + lo, :, sl[1]] += v
            return c
        kpart[...] = jnp.zeros(kpart.shape, F32)
        with jax.named_scope('kgen'):
            lax.fori_loop(0, 5 * 16, tile, 0)
        kq = jnp.sum(kpart[...], axis=1)[:, :D].astype(BF16)
        cpe.wait()
        for c in range(NF // TF):
            kf_s[c * TF:(c + 1) * TF, :] = _dot(fe_v[c * TF:(c + 1) * TF, :], kq).astype(BF16)
    pl.run_scoped(kgen, pltpu.VMEM((J, 8, DP), F32), pltpu.VMEM((NF, J), BF16))

    with jax.named_scope('dft'):
        fwd_dft(uf_s)
        spec_prod(uf_s, kf_s, False, True)
        inv_dft()
    dsk = dsk_ref[...].astype(F32)
    yb = acc_ld(allr).astype(BF16).astype(F32) + (u_s[...].astype(F32) * dsk).astype(BF16).astype(F32)
    hh = (x_ref[...].astype(F32) + yb.astype(BF16).astype(F32)).astype(BF16)
    h_s[...] = hh
    b_s[...] = _ln(hh.astype(F32))[0].astype(BF16)

    for c_ in wcp:
        c_.wait()
    def mlp(pre_s, z2_s, r2_s, dg_s, dwo_s, ob1, ob2):
        def rows(i):
            return pl.ds(pl.multiple_of(i * TM, TM), TM)

        def pa(i, c):
            r = rows(i)
            pre = _dot(b_s[r, :], win_ref[...]).astype(BF16)
            pre_s[r, :] = pre
            z2 = _gelu_and_grad(pre[:, FH:].astype(F32))[0].astype(BF16).astype(F32)
            z2n, r2 = _ln(z2)
            z2_s[r, :] = z2n.astype(BF16)
            r2_s[r, :] = r2
            return c
        with jax.named_scope('pa'):
            lax.fori_loop(0, L // TM, pa, 0)

        def pb(i, c):
            r = rows(i)
            g = (_dot(wsp_ref[r, :], z2_s[...]).astype(BF16).astype(F32)
                 + bsp_ref[r, :].astype(F32)).astype(BF16).astype(F32)
            z1, gp1 = _gelu_and_grad(pre_s[r, 0:FH].astype(F32))
            z1 = z1.astype(BF16).astype(F32)
            zg = (z1 * g).astype(BF16)
            go = go_ref[r, :]
            h2_ref[r, :] = (h_s[r, :].astype(F32)
                            + _dot_nt(zg, wout_ref[...]).astype(BF16).astype(F32)).astype(BF16)
            dzg = _dot(go, wout_ref[...]).astype(BF16).astype(F32)
            dwo_s[...] = jnp.where(i == 0, 0.0, dwo_s[...]) + _dot(got_ref[:, r], zg)
            dg = dzg * z1
            dbsp_ref[r, :] = jnp.sum(dg, axis=-1, keepdims=True).astype(BF16)
            dgb = dg.astype(BF16)
            dg_s[r, :] = dgb
            dwsp = _dot_nt(dgb, z2_s[...]).astype(BF16)

            @pl.when(i > 0)
            def _():
                pltpu.make_async_copy(ob1, dwsp_ref.at[r], sems.at[2]).wait()
            ob1[...] = dwsp
            pltpu.make_async_copy(ob1, dwsp_ref.at[r], sems.at[2]).start()
            pre_s[r, 0:FH] = (dzg * g * gp1).astype(BF16)
            return c
        with jax.named_scope('pb'):
            lax.fori_loop(0, L // TM, pb, 0)
        pltpu.make_async_copy(ob1, dwsp_ref.at[pl.ds(0, TM)], sems.at[2]).wait()
        dwout_ref[...] = dwo_s[...].astype(BF16)

        def pc(i, c):
            r = rows(i)
            dz2 = _dot_tn(wsp_ref[:, r], dg_s[...])
            dzz = _ln_bwd(dz2, z2_s[r, :].astype(F32), r2_s[r, :])
            gp2 = _gelu_and_grad(pre_s[r, FH:FF].astype(F32))[1]
            pre_s[r, FH:FF] = (dzz * gp2).astype(BF16)
            db = _dot_nt(pre_s[r, :], win_ref[...])
            bh, rh = _ln(h_s[r, :].astype(F32))
            dh_s[r, :] = (go_ref[r, :].astype(F32) + _ln_bwd(db, bh, rh)).astype(BF16)
            return c
        with jax.named_scope('pc'):
            lax.fori_loop(0, L // TM, pc, 0)

        def pd(i, c):
            cs = pl.ds(pl.multiple_of(i * 512, 512), 512)
            dwin = _dot_tn(b_s[...], pre_s[:, cs]).astype(BF16)

            @pl.when(i > 0)
            def _():
                pltpu.make_async_copy(ob2, dwin_ref.at[:, cs], sems.at[2]).wait()
            ob2[...] = dwin
            pltpu.make_async_copy(ob2, dwin_ref.at[:, cs], sems.at[2]).start()
            return c
        with jax.named_scope('pd'):
            lax.fori_loop(0, FF // 512, pd, 0)
        pltpu.make_async_copy(ob2, dwin_ref.at[:, pl.ds(0, 512)], sems.at[2]).wait()

    pl.run_scoped(mlp, pltpu.VMEM((L, FF), BF16), pltpu.VMEM((L, FH), BF16), pltpu.VMEM((L, 1), F32),
                  pltpu.VMEM((L, FH), BF16), pltpu.VMEM((D, FH), F32), pltpu.VMEM((TM, L), BF16), pltpu.VMEM((D, 512), BF16))

    def ssm_bwd(dyf_s, dkq_s, g_s, fet_v):
        cpe = pltpu.make_async_copy(fet_ref, fet_v, sems.at[2])
        cpe.start()
        acc_st(allr, dh_s[...].astype(F32))
        fwd_dft(dyf_s)
        spec_prod(dyf_s, uf_s, True, False)
        dkq_s[...] = jnp.zeros((J, DP), F32)
        cpe.wait()
        dkq_s[:, 0:D] = _dot(fet_v[...], yw_s[...])
        spec_prod(dyf_s, kf_s, True, True)
        inv_dft()
        dh = dh_s[...].astype(F32)
        uu = u_s[...].astype(F32)
        ddsk_ref[...] = jnp.sum(dh * uu, axis=0, keepdims=True).astype(BF16)
        du = acc_ld(allr) + dh * dsk
        _, rx = _ln(x_ref[...].astype(F32))
        dx_ref[...] = (dh + _ln_bwd(du, uu, rx)).astype(BF16)

        def tile(it, c):
            dt, nt = it // 16, it % 16
            sl, ar, ai, cbr, cbi = params(nt, dt)
            z = jnp.zeros_like(ar)
            g0r, g0i, g1r, g1i = z, z, z, z
            for b, s, hi, ys, (xr, xi) in _blocks(ar, ai, z + 1.0, z):
                tr, ti, tpr, tpi = dkq_s[pl.ds(b * 16, 1), sl[1]] + z, z, z, z
                for lo in range(1, len(ys)):
                    dk = dkq_s[pl.ds(b * 16 + lo, 1), sl[1]]
                    yr, yi = ys[lo]
                    dl = dk * float(lo << s)
                    tr, ti = tr + dk * yr, ti + dk * yi
                    tpr, tpi = tpr + dl * yr, tpi + dl * yi
                qh = float((16 * hi) << s)
                pr, pi_ = _cmul(xr, xi, tr, ti)
                g0r, g0i = g0r + pr, g0i + pi_
                pr, pi_ = _cmul(xr, xi, qh * tr + tpr, qh * ti + tpi)
                g1r, g1i = g1r + pr, g1i + pi_
            g_s[0, sl[0], sl[1]] = g0r
            g_s[1, sl[0], sl[1]] = g0i
            g_s[2, sl[0], sl[1]] = g1r
            g_s[3, sl[0], sl[1]] = g1i
            return c
        with jax.named_scope('ggen'):
            lax.fori_loop(0, 5 * 16, tile, 0)

        dtv = jnp.exp(ldt_ref[...].astype(F32)).astype(BF16).astype(F32)
        are, aim = are_ref[...].astype(F32), aim_ref[...].astype(F32)
        bre, bim = bre_ref[...].astype(F32), bim_ref[...].astype(F32)
        cre, cim = cre_ref[...].astype(F32), cim_ref[...].astype(F32)
        dbr, dbi = dtv * bre, dtv * bim
        cbr, cbi = _cmul(cre, cim, dbr, dbi)
        dcbr, dcbi = g_s[0], -g_s[1]
        t_r, t_i = _cmul(cbr, cbi, g_s[2], g_s[3])
        dar, dai = t_r, -t_i
        dcr, dci = _cmul(dbr, -dbi, dcbr, dcbi)
        ddbr, ddbi = _cmul(cre, -cim, dcbr, dcbi)
        dare_ref[...] = (dtv * dar).astype(BF16)
        daim_ref[...] = (dtv * dai).astype(BF16)
        dbre_ref[...] = (dtv * ddbr).astype(BF16)
        dbim_ref[...] = (dtv * ddbi).astype(BF16)
        dcre_ref[...] = dcr.astype(BF16)
        dcim_ref[...] = dci.astype(BF16)
        ddt = jnp.sum(bre * ddbr + bim * ddbi + are * dar + aim * dai, axis=0, keepdims=True)
        dldt_ref[...] = (ddt * dtv).astype(BF16)

    pl.run_scoped(ssm_bwd, pltpu.VMEM((NF, D), BF16), pltpu.VMEM((J, DP), F32),
                  pltpu.VMEM((4, N, DP), F32), pltpu.VMEM((J, NF), BF16))


@jax.jit
def pallas_sequential_preLN__ssm_conv_s4__mixer_gmlp__prompt_kernel(
    A_u, A_A_re, A_A_im, A_B_re, A_B_im, A_C_re, A_C_im, A_log_dt, A_Dskip,
    B_x, B_w_in, B_w_sp, B_b_sp, B_w_out, grad_out,
):
    fm, fe, fet = _consts()
    tp = lambda a: jnp.pad(a.T, ((0, 0), (0, DP - D)))
    ins = (A_u.reshape(L, D), grad_out.reshape(L, D), tp(A_A_re), tp(A_A_im), tp(A_B_re), tp(A_B_im),
           tp(A_C_re), tp(A_C_im), jnp.pad(A_log_dt.reshape(1, D), ((0, 0), (0, DP - D))),
           A_Dskip.reshape(1, D), B_w_in, B_w_sp, B_b_sp.reshape(L, 1), B_w_out.T, grad_out.reshape(L, D).T, fm, fe, fet)
    vm = pl.BlockSpec(memory_space=pltpu.VMEM)
    an = pl.BlockSpec(memory_space=pl.ANY)
    in_specs = [vm] * 10 + [an, an, vm, an, an, vm, an, an]
    out_specs = tuple([vm] * 10 + [an, an, vm, vm])
    sd = jax.ShapeDtypeStruct
    out_shape = (sd((L, D), BF16), sd((L, D), BF16)) + (sd((N, DP), BF16),) * 6 + (
        sd((1, DP), BF16), sd((1, D), BF16), sd((D, FF), BF16), sd((L, L), BF16), sd((L, 1), BF16),
        sd((D, FH), BF16))
    outs = pl.pallas_call(
        _kernel,
        out_shape=out_shape,
        in_specs=in_specs,
        out_specs=out_specs,
        scratch_shapes=[
            pltpu.VMEM((L, D), BF16), pltpu.VMEM((L, D), BF16), pltpu.VMEM((L, D), BF16),
            pltpu.VMEM((L, D), BF16), pltpu.VMEM((NF, D), BF16), pltpu.VMEM((NF, D), BF16),
            pltpu.VMEM((NF, D), BF16), pltpu.VMEM((5, L, 128), F32),
            pltpu.SemaphoreType.DMA((7,)),
            pltpu.VMEM((D, FF), BF16), pltpu.VMEM((L, L), BF16), pltpu.VMEM((D, FH), BF16),
            pltpu.VMEM((D, L), BF16),
        ],
        compiler_params=pltpu.CompilerParams(vmem_limit_bytes=127 * 1024 * 1024),
    )(*ins)
    h2, dx, dare, daim, dbre, dbim, dcre, dcim, dldt, ddsk, dwin, dwsp, dbsp, dwout = outs
    ut = lambda a: a[:, :D].T
    return (h2.reshape(1, L, D), dx.reshape(1, L, D), ut(dare), ut(daim), ut(dbre), ut(dbim), ut(dcre),
            ut(dcim), dldt[0, :D], ddsk.reshape(D), dwin, dwsp, dbsp.reshape(L), dwout.T)
```
